```python
import os as _os
_os.environ.setdefault("JAX_PLATFORMS", "cpu")
import jax
import jax.numpy as jnp

def _softmax(x, axis=-1):
    return jax.nn.softmax(x, axis=axis)
def _gelu(x):
    return jax.nn.gelu(x, approximate=True)
def _silu(x):
    return jax.nn.silu(x)
def _sigmoid(x):
    return jax.nn.sigmoid(x)
def _layernorm(x, axis=-1, eps=1e-5):
    m = jnp.mean(x, axis=axis, keepdims=True)
    v = jnp.var(x, axis=axis, keepdims=True)
    return (x - m) / jnp.sqrt(v + eps)
def _scatter_add(tgt, idx, src, axis=0):
    return tgt.at[idx].add(src)
def _segment_sum(src, seg, n):
    return jax.ops.segment_sum(src, seg, n)
class _Rng:
    def __init__(self, key):
        self._k = key
    def _next(self):
        self._k, sub = jax.random.split(self._k)
        return sub
    def normal(self, shape):
        return jax.random.normal(self._next(), shape, dtype=jnp.bfloat16)
    def randint(self, lo, hi, shape):
        return jax.random.randint(self._next(), shape, lo, hi, dtype=jnp.int32)
    def uniform(self, shape, lo=0.0, hi=1.0):
        return jax.random.uniform(self._next(), shape, jnp.bfloat16, lo, hi)
    def permutation(self, n):
        return jax.random.permutation(self._next(), n)


kernel_name = 'standalone__softmax_full_bidir__sampling'

def setup_inputs():
    _rng = _Rng(jax.random.key(int.from_bytes(__import__("os").urandom(4), "little")))
    _w = (lambda a: (lambda t: t.astype(jnp.bfloat16) if jnp.issubdtype(t.dtype, jnp.floating) else t)(jnp.asarray(a)))
    B, H, Sq, Skv, Dh = 8, 32, 1, 4096, 192
    return {
        "q": _w((lambda *s: _rng.normal(s) * 0.4)(B, H, Sq, Dh)),
        "k": _w((lambda *s: _rng.normal(s) * 0.4)(B, H, Skv, Dh)),
        "v": _w((lambda *s: _rng.normal(s) * 0.05)(B, H, Skv, Dh)),
    }

def reference(q, k, v):
    scale = q.shape[-1] ** -0.5
    scores = jnp.einsum('bhqd,bhkd->bhqk', q, k) * scale
    attn = _softmax(scores, axis=-1)
    return jnp.einsum('bhqk,bhkd->bhqd', attn, v)
```

```python
import jax
import jax.numpy as jnp
from jax import lax
import jax.experimental.pallas as pl
import jax.experimental.pallas.tpu as pltpu

_NBUF = 4
_PIECE = 128


@jax.jit
def pallas_standalone__softmax_full_bidir__sampling_kernel(
    q: jax.Array,
    k: jax.Array,
    v: jax.Array,
):
    B, H, Sq, D = q.shape
    S = k.shape[2]
    N = B * H
    scale = D ** -0.5

    def kernel(q_ref, k_hbm, v_hbm, o_ref, kbuf, vbuf, qf, acc, sems):
        qf[...] = q_ref[...].astype(jnp.float32)

        def start(src, dst, t, i, slot):
            for j in range(S // _PIECE):
                pltpu.make_async_copy(
                    src.at[i, :, pl.ds(j * _PIECE, _PIECE)],
                    dst.at[slot, :, pl.ds(j * _PIECE, _PIECE)],
                    sems.at[t, slot]).start(priority=j % 2)

        def wait(dst, t, slot):
            pltpu.make_async_copy(dst.at[slot], dst.at[slot], sems.at[t, slot]).wait()

        def prologue(i, c):
            start(k_hbm, kbuf, 0, i, i)
            start(v_hbm, vbuf, 1, i, i)
            return c
        lax.fori_loop(0, _NBUF - 1, prologue, 0)

        def body(i, c):
            slot = lax.rem(i, _NBUF)
            nslot = lax.rem(i + _NBUF - 1, _NBUF)
            more = i + _NBUF - 1 < N

            @pl.when(more)
            def _():
                start(k_hbm, kbuf, 0, i + _NBUF - 1, nslot)
            wait(kbuf, 0, slot)
            qi = jnp.broadcast_to(qf[pl.ds(i, 1), :], (8, D)).astype(k.dtype)
            s = jnp.dot(qi, kbuf[slot], preferred_element_type=jnp.float32) * scale
            m = jnp.max(s, axis=-1, keepdims=True)
            p = jnp.exp(s - m)
            l = jnp.sum(p, axis=-1, keepdims=True)

            @pl.when(more)
            def _():
                start(v_hbm, vbuf, 1, i + _NBUF - 1, nslot)
            wait(vbuf, 1, slot)
            o = lax.dot_general(p.astype(v.dtype), vbuf[slot], (((1,), (1,)), ((), ())),
                                preferred_element_type=jnp.float32)
            acc[pl.ds(i, 1), :] = (o / l)[0:1]
            return c
        lax.fori_loop(0, N, body, 0)
        o_ref[...] = acc[...].astype(o_ref.dtype)

    kt = jnp.swapaxes(k, 2, 3).reshape(N, D, S)
    vt = jnp.swapaxes(v, 2, 3).reshape(N, D, S)
    out = pl.pallas_call(
        kernel,
        out_shape=jax.ShapeDtypeStruct((N, D), q.dtype),
        in_specs=[pl.BlockSpec(memory_space=pltpu.VMEM),
                  pl.BlockSpec(memory_space=pl.ANY),
                  pl.BlockSpec(memory_space=pl.ANY)],
        out_specs=pl.BlockSpec(memory_space=pltpu.VMEM),
        scratch_shapes=[pltpu.VMEM((_NBUF, D, S), k.dtype),
                        pltpu.VMEM((_NBUF, D, S), v.dtype),
                        pltpu.VMEM((N, D), jnp.float32),
                        pltpu.VMEM((N, D), jnp.float32),
                        pltpu.SemaphoreType.DMA((2, _NBUF))],
        compiler_params=pltpu.CompilerParams(
            vmem_limit_bytes=100 * 1024 * 1024, disable_bounds_checks=True),
    )(q.reshape(N, D), kt, vt)
    return out.reshape(B, H, Sq, D)
```

```python
import numpy as np
import jax
import jax.numpy as jnp
from jax import lax
import jax.experimental.pallas as pl
import jax.experimental.pallas.tpu as pltpu


def make(L=4, NS=None, A=3, RMUL=11, NSEG=16, flags=None, HS=0, nocompute=False, wmode='each'):
    NS = NS or L + 1
    def fn(q, k, v):
        B, H, Sq, D = q.shape
        S = k.shape[2]
        N = B * H
        G = 8
        R = D // 8
        U = R // 2
        NG = N // G
        scale = D ** -0.5
        C0 = A * 128
        CW = S // NSEG
        PPS = 16 // NSEG

        def kernel(q_hbm, k_hbm, v_hbm, o_hbm, ring, qv, qb, et, s_acc, p_ref, r_ref, ov, sems, qsem, osem):
            def issuer(src, g, u, slot):
                bands = [lax.rem((2 * u + t) * RMUL, R) + g * (G * R) for t in range(2)]
                def piece(i):
                    b = bands[i // G] + (i % G) * R
                    pltpu.make_async_copy(src.at[b, :, pl.ds(0, C0)], ring.at[slot, pl.ds(8 * i, 8), pl.ds(0, C0)],
                                          sems.at[slot]).start(priority=0)
                    pltpu.make_async_copy(src.at[b, :, pl.ds(C0, S - C0)], ring.at[slot, pl.ds(8 * i, 8), pl.ds(C0, S - C0)],
                                          sems.at[slot]).start(priority=1)
                return piece

            def wait(slot):
                pltpu.make_async_copy(ring.at[slot], ring.at[slot], sems.at[slot]).wait()

            def nxt(slot):
                return lax.select(slot == NS - 1, 0, slot + 1)

            qcp = pltpu.make_async_copy(q_hbm, qv, qsem)

            def pro(u, c):
                piece = issuer(k_hbm, 0, u, u)
                for i in range(16):
                    piece(i)
                @pl.when(u == 0)
                def _():
                    qcp.start()
                return c
            lax.fori_loop(0, L, pro, 0)

            lane = lax.broadcasted_iota(jnp.int32, (1, 128), 1)
            drow = lax.broadcasted_iota(jnp.int32, (D, 128), 0)
            def mk(u, c):
                b0 = lax.rem(2 * u * RMUL, R); b1 = lax.rem((2 * u + 1) * RMUL, R)
                dsel = jnp.where(lane < 64, b0, b1) * 8 + (lane & 7)
                et[u] = jnp.where(drow == dsel, 1.0, 0.0).astype(jnp.bfloat16)
                return c
            lax.fori_loop(0, U, mk, 0)
            qcp.wait()

            own = lax.broadcasted_iota(jnp.int32, (G, 128), 0) == ((lax.broadcasted_iota(jnp.int32, (G, 128), 1) >> 3) & 7)

            def k_unit(g, u, slot, piece):
                x = jnp.dot(qv[g], et[u], preferred_element_type=jnp.float32)
                lhs = jnp.where(own, x, 0.0).astype(jnp.bfloat16)
                wait(slot)
                for j in range(NSEG):
                    cs = slice(j * CW, (j + 1) * CW)
                    if not nocompute:
                        s_acc[:, cs] += jnp.dot(lhs, ring[slot, :, cs], preferred_element_type=jnp.float32)
                    for i in range(j * PPS, (j + 1) * PPS):
                        piece(i)

            def v_unit(u, slot, piece, inv):
                wait(slot)
                r = None
                for j in range(NSEG):
                    cs = slice(j * CW, (j + 1) * CW)
                    if not nocompute or j == 0:
                        t = lax.dot_general(p_ref[:, cs], ring[slot, :, cs], (((1,), (1,)), ((), ())), preferred_element_type=jnp.float32)
                        r = t if r is None else r + t
                    for i in range(j * PPS, (j + 1) * PPS):
                        piece(i)
                rn = jnp.where(own, r * inv, 0.0).astype(jnp.bfloat16)
                r_ref[...] += lax.dot_general(rn, et[u], (((1,), (1,)), ((), ())), preferred_element_type=jnp.float32)

            def run(lo, hi, carry, unit, src, ig, du):
                def body(u, c):
                    slot, islot = c
                    piece = issuer(src, ig, u + du, islot) if src is not None else (lambda i: None)
                    unit(u, slot, piece)
                    return nxt(slot), nxt(islot)
                return lax.fori_loop(lo, hi, body, carry)

            def group(g, c):
                s_acc[...] = jnp.zeros_like(s_acc)
                r_ref[...] = jnp.zeros_like(r_ref)
                kc = lambda u, slot, piece: k_unit(g, u, slot, piece)
                c = run(0, U - L, c, kc, k_hbm, g, L)
                c = run(U - L, U, c, kc, v_hbm, g, L - U)
                s = s_acc[...] * scale
                m = jnp.max(s, axis=-1, keepdims=True)
                p = jnp.exp(s - m)
                inv = 1.0 / jnp.sum(p, axis=-1, keepdims=True)
                p_ref[...] = p.astype(p_ref.dtype)
                vc = lambda u, slot, piece: v_unit(u, slot, piece, inv)
                c = run(0, U - L, c, vc, v_hbm, g, L)
                mid = jnp.where(g + 1 < NG, U, U - L)
                c = run(U - L, mid, c, vc, k_hbm, g + 1, L - U)
                c = run(mid, U, c, vc, None, 0, 0)
                ov[g] = r_ref[...].astype(ov.dtype)
                if wmode == 'each':
                    pltpu.make_async_copy(ov.at[g], o_hbm.at[g], osem).start()
                elif wmode == 'two':
                    @pl.when(g == NG - 2)
                    def _():
                        pltpu.make_async_copy(ov.at[pl.ds(0, NG - 1)], o_hbm.at[pl.ds(0, NG - 1)], osem).start()
                return c
            lax.fori_loop(0, NG, group, (0, L))
            if wmode == 'two':
                pltpu.make_async_copy(ov.at[NG - 1], o_hbm.at[NG - 1], osem).start()
            elif wmode == 'end':
                pltpu.make_async_copy(ov, o_hbm, osem).start()
            pltpu.make_async_copy(ov, o_hbm, osem).wait()

        kt = jnp.swapaxes(k, 2, 3).reshape(N * R, 8, S)
        vt = jnp.swapaxes(v, 2, 3).reshape(N * R, 8, S)
        anyspec = pl.BlockSpec(memory_space=pl.ANY)
        out = pl.pallas_call(
            kernel,
            out_shape=jax.ShapeDtypeStruct((NG, G, D), q.dtype),
            in_specs=[anyspec, anyspec, anyspec],
            out_specs=anyspec,
            scratch_shapes=[pltpu.VMEM((NS, 128, S), k.dtype),
                            pltpu.VMEM((NG, G, D), q.dtype),
                            pltpu.VMEM((U, N, 128), jnp.float32),
                            pltpu.VMEM((U, D, 128), jnp.bfloat16),
                            pltpu.VMEM((G, S), jnp.float32),
                            pltpu.VMEM((G, S), v.dtype),
                            pltpu.VMEM((G, D), jnp.float32),
                            pltpu.VMEM((NG, G, D), q.dtype),
                            pltpu.SemaphoreType.DMA((NS,)),
                            pltpu.SemaphoreType.DMA(()),
                            pltpu.SemaphoreType.DMA(())],
            compiler_params=pltpu.CompilerParams(vmem_limit_bytes=64 * 1024 * 1024, disable_bounds_checks=True, flags=flags),
        )(q.reshape(NG, G, D), kt, vt)
        return out.reshape(B, H, Sq, D)
    return fn


_impl = make(3, wmode='end')


@jax.jit
def pallas_standalone__softmax_full_bidir__sampling_kernel(q, k, v):
    return _impl(q, k, v)
```

```python
import numpy as np
import jax
import jax.numpy as jnp
from jax import lax
import jax.experimental.pallas as pl
import jax.experimental.pallas.tpu as pltpu


def make(L=2, SETS=(4, 3, 4, 3, 4, 3), NSEG=2, flags=None, wmode="end", nocompute=False):
    NS = L + 1
    def fn(q, k, v):
        B, H, Sq, D = q.shape
        S = k.shape[2]
        N = B * H
        G = 16
        R = D // 8
        U = G
        NG = N // G
        NC = 4
        CW = S // NC
        NZ = R - sum(SETS)
        ZW = CW // 2
        scale = D ** -0.5
        starts = [sum(SETS[:i]) for i in range(len(SETS))]
        assert len(SETS) == 2 * NZ

        def kernel(q_hbm, k_hbm, v_hbm, o_hbm, ring, qv, et, s_acc, p_ref, ov, sems, qsem, osem):
            def issuer(src, g, u, slot):
                def piece(c, i):
                    z = R - NZ + i % NZ
                    zc = pl.ds(c * CW + (i // NZ) * ZW, ZW)
                    pltpu.make_async_copy(src.at[g * R + z, u, :, zc], ring.at[slot, z, :, zc],
                                          sems.at[slot, c]).start(priority=0)
                    cc = pl.ds(c * CW, CW)
                    pltpu.make_async_copy(src.at[pl.ds(g * R + starts[i], SETS[i]), u, :, cc],
                                          ring.at[slot, pl.ds(starts[i], SETS[i]), :, cc],
                                          sems.at[slot, c]).start(priority=1)
                return piece

            def wait(slot, c):
                x = ring.at[slot, :, :, pl.ds(c * CW, CW)]
                pltpu.make_async_copy(x, x, sems.at[slot, c]).wait()

            def nxt(slot):
                return lax.select(slot == NS - 1, 0, slot + 1)

            qcp = pltpu.make_async_copy(q_hbm, qv, qsem)

            def pro(u, c):
                piece = issuer(k_hbm, 0, u, u)
                for cc in range(NC):
                    for i in range(len(SETS)):
                        piece(cc, i)
                @pl.when(u == 0)
                def _():
                    qcp.start()
                return c
            lax.fori_loop(0, L, pro, 0)

            lane = lax.broadcasted_iota(jnp.int32, (1, D), 1)
            band0 = (lane >> 3) * U
            drow = lax.broadcasted_iota(jnp.int32, (D, D), 0)
            def mk(u, c):
                dsel = lax.rem(band0 + u, R) * 8 + (lane & 7)
                et[u] = jnp.where(drow == dsel, 1.0, 0.0).astype(jnp.bfloat16)
                return c
            lax.fori_loop(0, U, mk, 0)
            qcp.wait()

            rel = band0 - lax.broadcasted_iota(jnp.int32, (G, D), 0) * R
            def own(u):
                t = rel + u
                return (t >= 0) & (t < R)

            PPS = len(SETS) // NSEG
            SW = CW // NSEG

            def load(slot, c0):
                return ring[slot, :, :, pl.ds(c0, SW)].reshape(D, SW)

            def k_unit(g, u, slot, piece, carry):
                x = jnp.dot(qv[g], et[u], preferred_element_type=jnp.float32)
                lhs = jnp.where(own(u), x, 0.0).astype(jnp.bfloat16)
                for c in range(NC):
                    wait(slot, c)
                    for j in range(NSEG):
                        c0 = c * CW + j * SW
                        if not nocompute:
                            s_acc[:, c0:c0 + SW] += jnp.dot(lhs, load(slot, c0), preferred_element_type=jnp.float32)
                        for i in range(j * PPS, (j + 1) * PPS):
                            piece(c, i)
                return carry

            def v_unit(u, slot, piece, inv, out):
                r = None
                for c in range(NC):
                    wait(slot, c)
                    for j in range(NSEG):
                        c0 = c * CW + j * SW
                        if not nocompute or r is None:
                            t = lax.dot_general(p_ref[:, c0:c0 + SW], load(slot, c0), (((1,), (1,)), ((), ())), preferred_element_type=jnp.float32)
                            r = t if r is None else r + t
                        for i in range(j * PPS, (j + 1) * PPS):
                            piece(c, i)
                rn = jnp.where(own(u), r * inv, 0.0).astype(jnp.bfloat16)
                return out + lax.dot_general(rn, et[u], (((1,), (1,)), ((), ())), preferred_element_type=jnp.float32)

            def run(lo, hi, carry, unit, src, ig, du):
                def body(u, c):
                    slot, islot, x = c
                    piece = issuer(src, ig, u + du, islot) if src is not None else (lambda c, i: None)
                    x = unit(u, slot, piece, x)
                    return nxt(slot), nxt(islot), x
                return lax.fori_loop(lo, hi, body, carry)

            def group(g, c):
                s_acc[...] = jnp.zeros_like(s_acc)
                kc = lambda u, slot, piece, x: k_unit(g, u, slot, piece, x)
                c = run(0, U - L, c + (0,), kc, k_hbm, g, L)
                c = run(U - L, U, c, kc, v_hbm, g, L - U)
                s = s_acc[...] * scale
                m = jnp.max(s, axis=-1, keepdims=True)
                p = jnp.exp(s - m)
                inv = 1.0 / jnp.sum(p, axis=-1, keepdims=True)
                p_ref[...] = p.astype(p_ref.dtype)
                vc = lambda u, slot, piece, x: v_unit(u, slot, piece, inv, x)
                c = run(0, U - L, c[:2] + (jnp.zeros((G, D), jnp.float32),), vc, v_hbm, g, L)
                mid = jnp.where(g + 1 < NG, U, U - L)
                c = run(U - L, mid, c, vc, k_hbm, g + 1, L - U)
                if wmode == "late":
                    @pl.when(g == NG - 1)
                    def _():
                        pltpu.make_async_copy(ov.at[pl.ds(0, NG - 1)], o_hbm.at[pl.ds(0, NG - 1)], osem).start(priority=1)
                c = run(mid, U, c, vc, None, 0, 0)
                ov[g] = c[2].astype(ov.dtype)
                return c[:2]
            lax.fori_loop(0, NG, group, (0, L))
            if wmode == "late":
                pltpu.make_async_copy(ov.at[NG - 1], o_hbm.at[NG - 1], osem).start()
            else:
                pltpu.make_async_copy(ov, o_hbm, osem).start()
            pltpu.make_async_copy(ov, o_hbm, osem).wait()

        kt = jnp.swapaxes(k, 2, 3).reshape(NG * R, U, 8, S)
        vt = jnp.swapaxes(v, 2, 3).reshape(NG * R, U, 8, S)
        anyspec = pl.BlockSpec(memory_space=pl.ANY)
        out = pl.pallas_call(
            kernel,
            out_shape=jax.ShapeDtypeStruct((NG, G, D), q.dtype),
            in_specs=[anyspec, anyspec, anyspec],
            out_specs=anyspec,
            scratch_shapes=[pltpu.VMEM((NS, R, 8, S), k.dtype),
                            pltpu.VMEM((NG, G, D), q.dtype),
                            pltpu.VMEM((U, D, D), jnp.bfloat16),
                            pltpu.VMEM((G, S), jnp.float32),
                            pltpu.VMEM((G, S), v.dtype),
                            pltpu.VMEM((NG, G, D), q.dtype),
                            pltpu.SemaphoreType.DMA((NS, NC)),
                            pltpu.SemaphoreType.DMA(()),
                            pltpu.SemaphoreType.DMA(())],
            compiler_params=pltpu.CompilerParams(vmem_limit_bytes=32 * 1024 * 1024, disable_bounds_checks=True, flags=flags),
        )(q.reshape(NG, G, D), kt, vt)
        return out.reshape(B, H, Sq, D)
    return fn


_impl = make()


@jax.jit
def pallas_standalone__softmax_full_bidir__sampling_kernel(q, k, v):
    return _impl(q, k, v)
```

```python
import numpy as np
import jax
import jax.numpy as jnp
from jax import lax
import jax.experimental.pallas as pl
import jax.experimental.pallas.tpu as pltpu


def plan(layout, zrows, zparts):
    bulk, side, r = [], [], 0
    for x in layout:
        if x > 0:
            bulk.append((1, r, x, 0, 1))
        else:
            side += list(range(r, r - x, zrows))
        r += abs(x)
    side = [(0, z, zrows, j, zparts) for j in range(zparts) for z in side]
    out, k, acc, tot = [], 0, 0, sum(b[2] for b in bulk)
    for b in bulk:
        acc += b[2]
        t = int(round(acc * len(side) / tot))
        out += side[k:t] + [b]
        k = t
    return out, side


def make(L=3, layout=(-1, 3) * 6, z=(1, 1), lag=24, NSEG=2, flags=None, wmode="split", nocompute=False):
    NS = L + 1
    copies, side = plan(layout, *z)
    def fn(q, k, v):
        B, H, Sq, D = q.shape
        S = k.shape[2]
        N = B * H
        G = 16
        R = D // 8
        U = G
        NG = N // G
        NC = 4
        CW = S // NC
        SW = CW // NSEG
        scale = D ** -0.5
        nz = len(side)

        def schedule(c):
            out, j = [], 0
            for cp in copies:
                if cp[0] == 1:
                    out.append((0, c, cp))
                else:
                    n = c * nz + j - lag
                    du, rem = divmod(n, NC * nz)
                    out.append((du, rem // nz, side[rem % nz]))
                    j += 1
            return out
        sched = [schedule(c) for c in range(NC)]
        dus = sorted({d for s in sched for d, _, _ in s})

        def kernel(q_hbm, k_hbm, v_hbm, o_hbm, ring, qv, et, s_acc, p_ref, ov, sems, qsem, osem):
            def start(src, row0, u, slot, c, cp):
                prio, r, n, part, parts = cp
                cols = pl.ds(c * CW + part * (CW // parts), CW // parts)
                pltpu.make_async_copy(src.at[pl.ds(row0 + r, n), u, :, cols],
                                      ring.at[slot, pl.ds(r, n), :, cols],
                                      sems.at[slot, c]).start(priority=prio)

            def wait(slot, c):
                x = ring.at[slot, :, :, pl.ds(c * CW, CW)]
                pltpu.make_async_copy(x, x, sems.at[slot, c]).wait()

            qcp = pltpu.make_async_copy(q_hbm, qv, qsem)

            def pro(u, carry):
                for c in range(NC):
                    for du, cc, cp in sched[c]:
                        if du == 0:
                            start(k_hbm, 0, u, u, cc, cp)
                        else:
                            pl.when(u + du >= 0)(lambda: start(k_hbm, 0, u + du, u + du, cc, cp))
                pl.when(u == 0)(lambda: qcp.start())
                return carry
            lax.fori_loop(0, L, pro, 0)

            lane = lax.broadcasted_iota(jnp.int32, (1, D), 1)
            band0 = (lane >> 3) * U
            drow = lax.broadcasted_iota(jnp.int32, (D, D), 0)
            def mk(u, c):
                dsel = lax.rem(band0 + u, R) * 8 + (lane & 7)
                et[u] = jnp.where(drow == dsel, 1.0, 0.0).astype(jnp.bfloat16)
                return c
            lax.fori_loop(0, U, mk, 0)
            qcp.wait()

            rel = band0 - lax.broadcasted_iota(jnp.int32, (G, D), 0) * R
            def own(u):
                t = rel + u
                return (t >= 0) & (t < R)

            def load(slot, c0):
                return ring[slot, :, :, pl.ds(c0, SW)].reshape(D, SW)

            def prefetcher(cur, row_cur, nxt, row_nxt, nxt_ok, u, slot):
                tgt = {}
                for du in dus:
                    t = u + L + du
                    s = slot + (L + du)
                    tgt[du] = (t, jnp.where(s >= NS, s - NS, s), t < U, (t >= U) & nxt_ok)
                def go(c, j):
                    n = len(sched[c])
                    for du, cc, cp in sched[c][j * n // NSEG:(j + 1) * n // NSEG]:
                        t, s, here, there = tgt[du]
                        pl.when(here)(lambda: start(cur, row_cur, t, s, cc, cp))
                        pl.when(there)(lambda: start(nxt, row_nxt, t - U, s, cc, cp))
                return go

            def step(slot):
                return jnp.where(slot == NS - 1, 0, slot + 1)

            def group(g, slot):
                s_acc[...] = jnp.zeros_like(s_acc)

                def k_unit(u, slot):
                    go = prefetcher(k_hbm, g * R, v_hbm, g * R, True, u, slot)
                    x = jnp.dot(qv[g], et[u], preferred_element_type=jnp.float32)
                    lhs = jnp.where(own(u), x, 0.0).astype(jnp.bfloat16)
                    for c in range(NC):
                        wait(slot, c)
                        for j in range(NSEG):
                            c0 = c * CW + j * SW
                            if not nocompute:
                                s_acc[:, c0:c0 + SW] += jnp.dot(lhs, load(slot, c0), preferred_element_type=jnp.float32)
                            go(c, j)
                    return step(slot)
                slot = lax.fori_loop(0, U, k_unit, slot)

                s = s_acc[...] * scale
                m = jnp.max(s, axis=-1, keepdims=True)
                p = jnp.exp(s - m)
                inv = 1.0 / jnp.sum(p, axis=-1, keepdims=True)
                p_ref[...] = p.astype(p_ref.dtype)

                def v_unit(u, carry):
                    slot, out = carry
                    go = prefetcher(v_hbm, g * R, k_hbm, (g + 1) * R, g + 1 < NG, u, slot)
                    r = None
                    for c in range(NC):
                        wait(slot, c)
                        if c == NC - 1 and wmode == "split":
                            @pl.when((g == NG - 1) & (u == U - 1))
                            def _():
                                pltpu.make_async_copy(ov.at[pl.ds(0, NG - 1)], o_hbm.at[pl.ds(0, NG - 1)], osem).start()
                        for j in range(NSEG):
                            c0 = c * CW + j * SW
                            if not nocompute or r is None:
                                t = lax.dot_general(p_ref[:, c0:c0 + SW], load(slot, c0), (((1,), (1,)), ((), ())), preferred_element_type=jnp.float32)
                                r = t if r is None else r + t
                            go(c, j)
                    rn = jnp.where(own(u), r * inv, 0.0).astype(jnp.bfloat16)
                    out = out + lax.dot_general(rn, et[u], (((1,), (1,)), ((), ())), preferred_element_type=jnp.float32)
                    return step(slot), out
                slot, out = lax.fori_loop(0, U, v_unit, (slot, jnp.zeros((G, D), jnp.float32)))
                ov[g] = out.astype(ov.dtype)
                return slot
            lax.fori_loop(0, NG, group, 0)
            if wmode == "split":
                pltpu.make_async_copy(ov.at[NG - 1], o_hbm.at[NG - 1], osem).start()
            else:
                pltpu.make_async_copy(ov, o_hbm, osem).start()
            pltpu.make_async_copy(ov, o_hbm, osem).wait()

        kt = jnp.swapaxes(k, 2, 3).reshape(NG * R, U, 8, S)
        vt = jnp.swapaxes(v, 2, 3).reshape(NG * R, U, 8, S)
        anyspec = pl.BlockSpec(memory_space=pl.ANY)
        out = pl.pallas_call(
            kernel,
            out_shape=jax.ShapeDtypeStruct((NG, G, D), q.dtype),
            in_specs=[anyspec, anyspec, anyspec],
            out_specs=anyspec,
            scratch_shapes=[pltpu.VMEM((NS, R, 8, S), k.dtype),
                            pltpu.VMEM((NG, G, D), q.dtype),
                            pltpu.VMEM((U, D, D), jnp.bfloat16),
                            pltpu.VMEM((G, S), jnp.float32),
                            pltpu.VMEM((G, S), v.dtype),
                            pltpu.VMEM((NG, G, D), q.dtype),
                            pltpu.SemaphoreType.DMA((NS, NC)),
                            pltpu.SemaphoreType.DMA(()),
                            pltpu.SemaphoreType.DMA(())],
            compiler_params=pltpu.CompilerParams(vmem_limit_bytes=32 * 1024 * 1024, disable_bounds_checks=True, flags=flags),
        )(q.reshape(NG, G, D), kt, vt)
        return out.reshape(B, H, Sq, D)
    return fn


_impl = make(3, lag=26)


@jax.jit
def pallas_standalone__softmax_full_bidir__sampling_kernel(q, k, v):
    return _impl(q, k, v)
```

```python
import jax
import jax.numpy as jnp
from jax import lax
import jax.experimental.pallas as pl
import jax.experimental.pallas.tpu as pltpu

_HEADS = 8
_UNITS = 16
_CHUNKS = 4
_SET = 4
_AHEAD = 4
_SLOTS = _AHEAD + 1
_LAG = 26


@jax.jit
def pallas_standalone__softmax_full_bidir__sampling_kernel(
    q: jax.Array,
    k: jax.Array,
    v: jax.Array,
):
    B, H, Sq, D = q.shape
    S = k.shape[2]
    groups = B * H // _HEADS
    bands = D // 8
    rows = _HEADS * bands // _UNITS
    width = rows * 8
    pairs = rows // _SET
    cw = S // _CHUNKS
    scale = D ** -0.5
    assert Sq == 1 and groups * _HEADS == B * H and groups > 1
    assert pairs * _SET * _UNITS * 8 == _HEADS * D and S % (128 * _CHUNKS) == 0
    assert _LAG <= (_AHEAD - 1) * _CHUNKS * pairs

    def chunk_copies(c):
        copies = []
        for i in range(pairs):
            du, n = divmod(c * pairs + i - _LAG, _CHUNKS * pairs)
            copies.append((du, n // pairs, (n % pairs) * _SET, 1, 0))
            copies.append((0, c, i * _SET + 1, _SET - 1, 1))
        return copies

    def kernel(q_hbm, k_hbm, v_hbm, o_hbm,
               ring, q_vmem, sel, s_acc, p_vmem, o_vmem, sems, q_sem, o_sem):

        def start(src, row0, unit, slot, c, row, nrows, priority):
            cols = pl.ds(c * cw, cw)
            pltpu.make_async_copy(
                src.at[pl.ds(row0 + row, nrows), unit, :, cols],
                ring.at[slot, pl.ds(row, nrows), :, cols],
                sems.at[slot, c],
            ).start(priority=priority)

        def wait(slot, c):
            dst = ring.at[slot, :, :, pl.ds(c * cw, cw)]
            pltpu.make_async_copy(dst, dst, sems.at[slot, c]).wait()

        def load(slot, c):
            return ring[slot, :, :, pl.ds(c * cw, cw)].reshape(width, cw)

        def prefetcher(cur, cur_row, nxt, nxt_row, has_nxt, u, slot):
            targets = {}
            for c in range(_CHUNKS):
                for du, *_ in chunk_copies(c):
                    if du not in targets:
                        t, s = u + (_AHEAD + du), slot + (_AHEAD + du)
                        targets[du] = (t, jnp.where(s >= _SLOTS, s - _SLOTS, s),
                                       t < _UNITS, (t >= _UNITS) & has_nxt)

            def prefetch(c):
                for du, *copy in chunk_copies(c):
                    t, s, in_cur, in_nxt = targets[du]
                    pl.when(in_cur)(lambda: start(cur, cur_row, t, s, *copy))
                    pl.when(in_nxt)(lambda: start(nxt, nxt_row, t - _UNITS, s, *copy))
            return prefetch

        def next_slot(slot):
            return jnp.where(slot == _SLOTS - 1, 0, slot + 1)

        band0 = (lax.broadcasted_iota(jnp.int32, (1, width), 1) >> 3) * _UNITS
        in_band = lax.broadcasted_iota(jnp.int32, (1, width), 1) & 7
        feature = lax.broadcasted_iota(jnp.int32, (D, width), 0)
        band_in_head = band0 - lax.broadcasted_iota(jnp.int32, (_HEADS, width), 0) * bands

        def owns(u):
            b = band_in_head + u
            return (b >= 0) & (b < bands)

        q_copy = pltpu.make_async_copy(q_hbm, q_vmem, q_sem)

        @pl.loop(0, _AHEAD)
        def _(u):
            for c in range(_CHUNKS):
                for du, *copy in chunk_copies(c):
                    pl.when(u + du >= 0)(lambda: start(k_hbm, 0, u + du, u + du, *copy))
            pl.when(u == 0)(q_copy.start)

        @pl.loop(0, _UNITS)
        def _(u):
            held = lax.rem(band0 + u, bands) * 8 + in_band
            sel[u] = jnp.where(feature == held, 1.0, 0.0).astype(sel.dtype)

        q_copy.wait()

        contract_last = (((1,), (1,)), ((), ()))

        def group(g, slot):
            s_acc[...] = jnp.zeros_like(s_acc)

            def k_unit(u, slot):
                prefetch = prefetcher(k_hbm, g * rows, v_hbm, g * rows, True, u, slot)
                lhs = jnp.dot(q_vmem[g], sel[u], preferred_element_type=jnp.float32)
                lhs = jnp.where(owns(u), lhs, 0.0).astype(k.dtype)
                for c in range(_CHUNKS):
                    prefetch(c)
                    wait(slot, c)
                    s_acc[:, pl.ds(c * cw, cw)] += jnp.dot(
                        lhs, load(slot, c), preferred_element_type=jnp.float32)
                return next_slot(slot)

            slot = lax.fori_loop(0, _UNITS, k_unit, slot)

            s = s_acc[...] * scale
            p = jnp.exp(s - jnp.max(s, axis=-1, keepdims=True))
            inv = 1.0 / jnp.sum(p, axis=-1, keepdims=True)
            p_vmem[...] = p.astype(p_vmem.dtype)

            def v_unit(u, carry):
                slot, out = carry
                prefetch = prefetcher(
                    v_hbm, g * rows, k_hbm, (g + 1) * rows, g + 1 < groups, u, slot)
                acc = None
                for c in range(_CHUNKS):
                    prefetch(c)
                    wait(slot, c)
                    if c == _CHUNKS - 1:
                        @pl.when((g == groups - 1) & (u == _UNITS - 1))
                        def _():
                            done = pl.ds(0, groups - 1)
                            pltpu.make_async_copy(
                                o_vmem.at[done], o_hbm.at[done], o_sem).start()
                    part = lax.dot_general(
                        p_vmem[:, pl.ds(c * cw, cw)], load(slot, c), contract_last,
                        preferred_element_type=jnp.float32)
                    acc = part if acc is None else acc + part
                mine = jnp.where(owns(u), acc * inv, 0.0).astype(o_vmem.dtype)
                out = out + lax.dot_general(
                    mine, sel[u], contract_last, preferred_element_type=jnp.float32)
                return next_slot(slot), out

            slot, out = lax.fori_loop(
                0, _UNITS, v_unit, (slot, jnp.zeros((_HEADS, D), jnp.float32)))
            o_vmem[g] = out.astype(o_vmem.dtype)
            return slot

        lax.fori_loop(0, groups, group, 0)
        pltpu.make_async_copy(o_vmem.at[groups - 1], o_hbm.at[groups - 1], o_sem).start()
        pltpu.make_async_copy(o_vmem, o_hbm, o_sem).wait()

    def banded(x):
        return jnp.swapaxes(x, 2, 3).reshape(groups * rows, _UNITS, 8, S)

    in_hbm = pl.BlockSpec(memory_space=pl.ANY)
    out = pl.pallas_call(
        kernel,
        out_shape=jax.ShapeDtypeStruct((groups, _HEADS, D), q.dtype),
        in_specs=[in_hbm, in_hbm, in_hbm],
        out_specs=in_hbm,
        scratch_shapes=[
            pltpu.VMEM((_SLOTS, rows, 8, S), k.dtype),
            pltpu.VMEM((groups, _HEADS, D), q.dtype),
            pltpu.VMEM((_UNITS, D, width), q.dtype),
            pltpu.VMEM((_HEADS, S), jnp.float32),
            pltpu.VMEM((_HEADS, S), v.dtype),
            pltpu.VMEM((groups, _HEADS, D), q.dtype),
            pltpu.SemaphoreType.DMA((_SLOTS, _CHUNKS)),
            pltpu.SemaphoreType.DMA(()),
            pltpu.SemaphoreType.DMA(()),
        ],
        compiler_params=pltpu.CompilerParams(
            disable_bounds_checks=True, disable_semaphore_checks=True),
    )(q.reshape(groups, _HEADS, D), banded(k), banded(v))
    return out.reshape(B, H, Sq, D)
```
